```python
import jax
import jax.numpy as jnp

def _softmax(x, axis=-1):
    return jax.nn.softmax(x, axis=axis)
def _gelu(x):
    return jax.nn.gelu(x, approximate=True)
def _silu(x):
    return jax.nn.silu(x)
def _sigmoid(x):
    return jax.nn.sigmoid(x)
def _layernorm(x, axis=-1, eps=1e-5):
    m = jnp.mean(x, axis=axis, keepdims=True)
    v = jnp.var(x, axis=axis, keepdims=True)
    return (x - m) / jnp.sqrt(v + eps)
def _scatter_add(tgt, idx, src, axis=0):
    return tgt.at[idx].add(src)
def _segment_sum(src, seg, n):
    return jax.ops.segment_sum(src, seg, n)
class _Rng:
    def __init__(self, key):
        self._k = key
    def _next(self):
        self._k, sub = jax.random.split(self._k)
        return sub
    def normal(self, shape):
        return jax.random.normal(self._next(), shape, dtype=jnp.bfloat16)
    def randint(self, lo, hi, shape):
        return jax.random.randint(self._next(), shape, lo, hi, dtype=jnp.int32)
    def uniform(self, shape, lo=0.0, hi=1.0):
        return jax.random.uniform(self._next(), shape, jnp.bfloat16, lo, hi)
    def permutation(self, n):
        return jax.random.permutation(self._next(), n)


kernel_name = 'gated_mix__sliding_block_cached__mixer_s_mlp__decode'

def setup_inputs():
    _rng = _Rng(jax.random.key(int.from_bytes(__import__("os").urandom(4), "little")))
    _w = (lambda a: (lambda t: t.astype(jnp.bfloat16) if jnp.issubdtype(t.dtype, jnp.floating) else t)(jnp.asarray(a)))
    def _A_setup():
        B, Sq, D = 1, 1, 576
        Hq, Hkv, Sk, Dh = 32, 16, 65536, 128
        assert Hq % Hkv == 0, (Hq, Hkv)
        return {
            "x": _w((lambda *s: _rng.normal(s) * 0.05)(B, Sq, D)),
            "k_cache": _w((lambda *s: _rng.normal(s) * 0.05)(B, Hkv, Sk, Dh)),
            "v_cache": _w((lambda *s: _rng.normal(s) * 0.05)(B, Hkv, Sk, Dh)),
            "wq": _w((lambda *s: _rng.normal(s) * 0.05)(D, Hq * Dh) * (D ** -0.5)),
            "wo": _w((lambda *s: _rng.normal(s) * 0.05)(Hq * Dh, D) * ((Hq * Dh) ** -0.5)),
        }
    _A_in = _A_setup()

    def _B_setup():
        B, S, D, F = 1, 1, 576, 4608
        return {
            "x":  _w((lambda *s: _rng.normal(s) * 0.05)(B, S, D)),
            "w1": _w((lambda *s: _rng.normal(s) * 0.05)(D, D) * (D ** -0.5)),
            "w2": _w((lambda *s: _rng.normal(s) * 0.05)(D, D) * (D ** -0.5)),
            "w3": _w((lambda *s: _rng.normal(s) * 0.05)(D, F) * (D ** -0.5)),
            "w4": _w((lambda *s: _rng.normal(s) * 0.05)(F, D) * (F ** -0.5)),
        }
    _B_in = _B_setup()

    return {
        "A_x": _A_in["x"],
        "A_k_cache": _A_in["k_cache"],
        "A_v_cache": _A_in["v_cache"],
        "A_wq": _A_in["wq"],
        "A_wo": _A_in["wo"],
        "B_x": _B_in["x"],
        "B_w1": _B_in["w1"],
        "B_w2": _B_in["w2"],
        "B_w3": _B_in["w3"],
        "B_w4": _B_in["w4"],
        "gate_w": _w((lambda *s: _rng.normal(s) * 0.05)(576)),
    }

def reference(A_x, A_k_cache, A_v_cache, A_wq, A_wo, B_x, B_w1, B_w2, B_w3, B_w4, gate_w):
    def _A_ref(x, k_cache, v_cache, wq, wo):
        B, Sq, D = x.shape
        Hq, Dh = 32, 128
        Hkv, Sk = k_cache.shape[1], k_cache.shape[2]
        W = min(4096, max(256, Sk // 4))
        rep = Hq // Hkv
        q = (lambda x, *d: x.transpose(*d))((x @ wq).reshape(B, Sq, Hq, Dh), 0, 2, 1, 3)
        k = jnp.repeat(k_cache[:, :, Sk - W:, :], rep, axis=1)
        v = jnp.repeat(v_cache[:, :, Sk - W:, :], rep, axis=1)
        scores = jnp.einsum("bhqd,bhkd->bhqk", q, k) * (Dh ** -0.5)
        p = _softmax(scores, axis=-1)
        o = jnp.einsum("bhqk,bhkd->bhqd", p, v)
        return (lambda x, *d: x.transpose(*d))(o, 0, 2, 1, 3).reshape(B, Sq, Hq * Dh) @ wo

    def _B_ref(x, w1, w2, w3, w4):
        B, S, D = x.shape
        h = _gelu(_layernorm(x, axis=-1) @ w1)
        c = D // 4
        g0 = jnp.pad(h[:, :, 0*c:1*c], ((0, 0), (1, 0), (0, 0)))[:, :S, :]
        g1 = jnp.pad(h[:, :, 1*c:2*c], ((0, 0), (0, 1), (0, 0)))[:, 1:, :]
        g2 = jnp.pad(h[:, :, 2*c:3*c], ((0, 0), (2, 0), (0, 0)))[:, :S, :]
        g3 = jnp.pad(h[:, :, 3*c:   ], ((0, 0), (0, 2), (0, 0)))[:, 2:, :]
        hs = jnp.concatenate([g0, g1, g2, g3], axis=-1) @ w2
        x1 = x + hs
        h2 = _gelu(_layernorm(x1, axis=-1) @ w3) @ w4
        return x1 + h2

    x = A_x
    g = _sigmoid((x * gate_w).sum(-1, keepdims=True))
    a = _A_ref(x, A_k_cache, A_v_cache, A_wq, A_wo)
    b = _B_ref(x, B_w1, B_w2, B_w3, B_w4)
    return g * a + (1 - g) * b
```

```python
import functools

import jax
import jax.numpy as jnp
import jax.experimental.pallas as pl
import jax.experimental.pallas.tpu as pltpu

_HQ = 32
_DH = 128
_ROWS = 8
_NT = (((1,), (1,)), ((), ()))
_W4_ROW_CHUNKS = (256, 192, 128)


def _dot(a, b):
    return jnp.dot(a, b, preferred_element_type=jnp.float32)


def _dot_nt(a, b):
    return jax.lax.dot_general(a, b, _NT, preferred_element_type=jnp.float32)


def _kernel(
    x_hbm, gw_hbm, k_hbm, v_hbm, wq_hbm, wo_hbm, w3_hbm, w4_hbm,
    o_ref,
    x_v, gw_v, k_v, v_v, wq_v, wo_v, w3_v, w4_v, h_v, sems,
    *, window,
):
    n_kv, s_k = k_hbm.shape[1], k_hbm.shape[2]
    d_model, d_ff = w3_hbm.shape
    bf16, f32 = jnp.bfloat16, jnp.float32
    n_w4 = len(_W4_ROW_CHUNKS)

    def kv_copies(j):
        rows = pl.ds(s_k - window, window)
        return (
            pltpu.make_async_copy(k_hbm.at[0, j, rows, :], k_v.at[j], sems.at[4 + n_w4 + j]),
            pltpu.make_async_copy(v_hbm.at[0, j, rows, :], v_v.at[j], sems.at[4 + n_w4 + j]),
        )

    x_cp = pltpu.make_async_copy(x_hbm.at[0], x_v, sems.at[0])
    gw_cp = pltpu.make_async_copy(gw_hbm, gw_v, sems.at[0])
    w3_cp = pltpu.make_async_copy(w3_hbm, w3_v, sems.at[1])
    wq_cp = pltpu.make_async_copy(wq_hbm, wq_v, sems.at[2])
    wo_cp = pltpu.make_async_copy(wo_hbm, wo_v, sems.at[3])
    w4_cps, w4_rows, start = [], [], 0
    for i, n in enumerate(_W4_ROW_CHUNKS):
        rows = pl.ds(start, n)
        w4_cps.append(pltpu.make_async_copy(w4_hbm.at[rows, :], w4_v.at[rows, :], sems.at[4 + i]))
        w4_rows.append(rows)
        start += n

    w3_cp.start()
    x_cp.start()
    gw_cp.start()
    wq_cp.start()
    wo_cp.start()
    for j in range(n_kv):
        for cp in kv_copies(j):
            cp.start()
    for cp in w4_cps:
        cp.start()

    w3_cp.wait()
    x_cp.wait()
    gw_cp.wait()

    x = x_v[...].astype(f32)
    gw = gw_v[...].astype(f32).reshape(1, d_model)
    gate = jax.nn.sigmoid(jnp.sum(x * gw, axis=-1, keepdims=True))
    mean = jnp.mean(x, axis=-1, keepdims=True)
    xc = x - mean
    var = jnp.mean(xc * xc, axis=-1, keepdims=True)
    ln = xc / jnp.sqrt(var + 1e-5)
    ln8 = jnp.broadcast_to(ln, (_ROWS, d_model)).astype(bf16)
    x8 = jnp.broadcast_to(x, (_ROWS, d_model)).astype(bf16)

    ff_chunk = 512

    def ff_up(i, carry):
        cols = pl.ds(pl.multiple_of(i * ff_chunk, ff_chunk), ff_chunk)
        h_v[:, cols] = jax.nn.gelu(_dot(ln8, w3_v[:, cols]), approximate=True)
        return carry

    jax.lax.fori_loop(0, d_ff // ff_chunk, ff_up, None)

    wq_cp.wait()
    wo_cp.wait()
    even_row = jax.lax.broadcasted_iota(jnp.int32, (_ROWS, _DH), 0) % 2 == 0

    def head(j, acc):
        cols = pl.ds(pl.multiple_of(j * 2 * _DH, 2 * _DH), 2 * _DH)
        q = _dot(x8, wq_v[:, cols])
        q = jnp.where(even_row, q[:, :_DH], q[:, _DH:]).astype(bf16)
        for cp in kv_copies(j):
            cp.wait()
        s = _dot_nt(q, k_v[j]) * (_DH ** -0.5)
        p = jnp.exp(s - jnp.max(s, axis=-1, keepdims=True))
        denom = jnp.sum(p, axis=-1, keepdims=True)
        o = _dot(p.astype(bf16), v_v[j]) / denom
        o2 = jnp.concatenate(
            [jnp.broadcast_to(o[0:1], (_ROWS, _DH)), jnp.broadcast_to(o[1:2], (_ROWS, _DH))],
            axis=-1,
        )
        return acc + _dot_nt(o2.astype(bf16), wo_v[:, cols])

    attn = jax.lax.fori_loop(0, n_kv, head, jnp.zeros((_ROWS, d_model), f32))
    base = gate * attn[0:1] + (1.0 - gate) * x
    h = h_v[...].astype(bf16)

    start = 0
    for cp, rows, n in zip(w4_cps, w4_rows, _W4_ROW_CHUNKS):
        cp.wait()
        ff = _dot_nt(h, w4_v[rows, :])
        out = base[:, start:start + n] + (1.0 - gate) * ff[0:1]
        o_ref[0, :, start:start + n] = out.astype(o_ref.dtype)
        start += n


@jax.jit
def pallas_gated_mix__sliding_block_cached__mixer_s_mlp__decode_kernel(
    A_x: jax.Array,
    A_k_cache: jax.Array,
    A_v_cache: jax.Array,
    A_wq: jax.Array,
    A_wo: jax.Array,
    B_x: jax.Array,
    B_w1: jax.Array,
    B_w2: jax.Array,
    B_w3: jax.Array,
    B_w4: jax.Array,
    gate_w: jax.Array,
):
    del B_x, B_w1, B_w2
    batch, s_q, d_model = A_x.shape
    _, n_kv, s_k, d_head = A_k_cache.shape
    d_ff = B_w3.shape[1]
    assert (batch, s_q) == (1, 1) and d_head == _DH and _HQ == 2 * n_kv
    assert sum(_W4_ROW_CHUNKS) == d_model
    window = min(4096, max(256, s_k // 4))
    bf16 = jnp.bfloat16

    hbm = pl.BlockSpec(memory_space=pltpu.HBM)
    return pl.pallas_call(
        functools.partial(_kernel, window=window),
        out_shape=jax.ShapeDtypeStruct(A_x.shape, A_x.dtype),
        in_specs=[hbm] * 8,
        scratch_shapes=[
            pltpu.VMEM((1, d_model), bf16),
            pltpu.VMEM((d_model,), bf16),
            pltpu.VMEM((n_kv, window, d_head), bf16),
            pltpu.VMEM((n_kv, window, d_head), bf16),
            pltpu.VMEM((d_model, _HQ * _DH), bf16),
            pltpu.VMEM((d_model, _HQ * _DH), bf16),
            pltpu.VMEM((d_model, d_ff), bf16),
            pltpu.VMEM((d_model, d_ff), bf16),
            pltpu.VMEM((_ROWS, d_ff), jnp.float32),
            pltpu.SemaphoreType.DMA((4 + len(_W4_ROW_CHUNKS) + n_kv,)),
        ],
        compiler_params=pltpu.CompilerParams(vmem_limit_bytes=100 * 2**20),
    )(A_x, gate_w, A_k_cache, A_v_cache, A_wq, A_wo.T, B_w3, B_w4.T)
```

```python
import functools

import jax
import jax.numpy as jnp
from jax import lax
import jax.experimental.pallas as pl
import jax.experimental.pallas.tpu as pltpu

_HQ = 32
_LANES = 128
_ROWS = 8
_UNIT = 8
_NT = (((1,), (1,)), ((), ()))


def _dot(a, b):
    return jnp.dot(a, b, preferred_element_type=jnp.float32)


def _dot_nt(a, b):
    return lax.dot_general(a, b, _NT, preferred_element_type=jnp.float32)


def _aligned(i, n):
    start = i * n
    return pl.ds(start if isinstance(start, int) else pl.multiple_of(start, n), n)


def _kernel(
    x_hbm, gw_hbm, k_hbm, v_hbm, wq_hbm, wo_hbm, w3_hbm, w4_hbm,
    o_ref,
    x_v, gw_v, k_v, v_v, wq_v, wo_v, w3_v, w4_v, q_s, s_s, o_s, h_s,
    bulk_sem, side_sem, tail_sem,
    *, window, kv_side, w_side, tail_groups,
):
    n_kv, s_k = k_hbm.shape[1], k_hbm.shape[2]
    d_model, d_ff = w3_hbm.shape
    bf16, f32 = jnp.bfloat16, jnp.float32
    kv_step = window // _UNIT
    kv_bulk = kv_step - kv_side
    w_bulk = d_model - w_side
    n_q, n_ff = _HQ, d_ff // _LANES
    scale = _LANES ** -0.5

    def kv_copies(src, dst, j, s, par):
        def part(base, n, sem):
            off = base + s * n
            off = off if isinstance(off, int) else pl.multiple_of(off, 8)
            return pltpu.make_async_copy(
                src.at[0, j, pl.ds(s_k - window + off, n), :], dst.at[j, pl.ds(off, n), :], sem.at[par])
        return (lambda: part(0, kv_bulk, bulk_sem)), (lambda: part(_UNIT * kv_bulk, kv_side, side_sem))

    def w_copies(src, dst, t, par):
        cols = _aligned(t, _LANES)
        def part(lo, n, sem):
            return pltpu.make_async_copy(src.at[pl.ds(lo, n), cols], dst.at[pl.ds(lo, n), cols], sem.at[par])
        return (lambda: part(0, w_bulk, bulk_sem)), (lambda: part(w_bulk, w_side, side_sem))

    def issue(copies):
        bulk, side = copies
        side().start(priority=0)
        bulk().start(priority=1)

    def land(copies):
        bulk, side = copies
        bulk().wait()
        side().wait()

    def parity(t):
        return (t // _UNIT) % 2 if isinstance(t, int) else lax.shift_right_logical(t, 3) & 1

    def w_stream(src, dst, par0):
        return lambda t: w_copies(src, dst, t, parity(t + par0 * _UNIT))

    def kv_stream(src, dst, j, par):
        return lambda s: kv_copies(src, dst, j, s, par)

    def shifted(fn, off):
        return lambda t, *rest: fn(t + off, *rest)

    def run(n, landing, issuing, compute=None, carry=None):
        def body(t, c):
            land(landing(t))
            if issuing is not None:
                issue(issuing(t))
            return c if compute is None else compute(t, c)
        return lax.fori_loop(0, n, body, carry)

    def tail_copy(g):
        cols = pl.ds(sum(tail_groups[:g]) * _LANES + d_ff - _UNIT * _LANES, tail_groups[g] * _LANES)
        return pltpu.make_async_copy(w4_hbm.at[:, cols], w4_v.at[:, cols], tail_sem.at[g])

    wq = w_stream(wq_hbm, wq_v, 0)
    wo = w_stream(wo_hbm, wo_v, 0)
    w3 = w_stream(w3_hbm, w3_v, 0)
    w4 = lambda t: w_copies(w4_hbm, w4_v, t, parity(t + n_ff))
    k_stream = lambda j: kv_stream(k_hbm, k_v, j, 0)
    v_stream = lambda j: kv_stream(v_hbm, v_v, j, 1)

    x_cp = pltpu.make_async_copy(x_hbm.at[0], x_v, tail_sem.at[0])
    gw_cp = pltpu.make_async_copy(gw_hbm, gw_v, tail_sem.at[0])
    wq(0)[0]().start(priority=1)
    x_cp.start()
    gw_cp.start()
    for t in range(1, _UNIT):
        wq(t)[0]().start(priority=1)
    for t in range(_UNIT):
        wq(t)[1]().start(priority=0)

    run(_UNIT, wq, shifted(wq, _UNIT))

    x_cp.wait()
    gw_cp.wait()
    x = x_v[...].astype(f32)
    gw = gw_v[...].astype(f32).reshape(1, d_model)
    gate = jax.nn.sigmoid(jnp.sum(x * gw, axis=-1, keepdims=True))
    xc = x - jnp.mean(x, axis=-1, keepdims=True)
    var = jnp.mean(xc * xc, axis=-1, keepdims=True)
    ln8 = jnp.broadcast_to(xc / jnp.sqrt(var + 1e-5), (_ROWS, d_model)).astype(bf16)
    x8 = jnp.broadcast_to(x, (_ROWS, d_model)).astype(bf16)

    def q_proj(t, c):
        q_s[t] = _dot(x8, wq_v[:, _aligned(t, _LANES)])
        return c

    even_row = lax.broadcasted_iota(jnp.int32, (_ROWS, _LANES), 0) % 2 == 0

    def lane_tiles(a):
        return [a[:, i:i + _LANES] for i in range(0, a.shape[1], _LANES)]

    def scores_unit(j, issuing):
        q = jnp.where(even_row, q_s[2 * j], q_s[2 * j + 1]).astype(bf16)

        def qk(s, m):
            sc = _dot_nt(q, k_v[j, _aligned(s, kv_step), :])
            s_s[s] = sc
            return functools.reduce(jnp.maximum, lane_tiles(sc), m)

        m = run(_UNIT, v_stream(j), issuing, qk, jnp.full((_ROWS, _LANES), -jnp.inf, f32))
        return jnp.max(m, axis=-1, keepdims=True)

    def values_unit(j, row_max, landing, issuing):
        def pv(s, c):
            denom, acc = c
            p = jnp.exp((s_s[s] - row_max) * scale)
            denom = functools.reduce(jnp.add, lane_tiles(p), denom)
            return denom, acc + _dot(p.astype(bf16), v_v[j, _aligned(s, kv_step), :])

        zero = jnp.zeros((_ROWS, _LANES), f32)
        denom, acc = run(_UNIT, landing, issuing, pv, (zero, zero))
        o = acc / jnp.sum(denom, axis=-1, keepdims=True)
        o_s[2 * j] = jnp.broadcast_to(o[0:1], (_ROWS, _LANES))
        o_s[2 * j + 1] = jnp.broadcast_to(o[1:2], (_ROWS, _LANES))

    def o_proj(t, acc):
        return acc + _dot_nt(o_s[t].astype(bf16), wo_v[:, _aligned(t, _LANES)])

    def ff_up(t, c):
        h_s[t] = jax.nn.gelu(_dot(ln8, w3_v[:, _aligned(t, _LANES)]), approximate=True)
        return c

    def ff_down(t, acc):
        return acc + _dot_nt(h_s[t].astype(bf16), w4_v[:, _aligned(t, _LANES)])

    u = _UNIT
    run(n_q - 2 * u, shifted(wq, u), shifted(wq, 2 * u), q_proj)
    run(u, shifted(wq, n_q - u), k_stream(0), shifted(q_proj, n_q - 2 * u))
    run(u, k_stream(0), v_stream(0), shifted(q_proj, n_q - u))

    def head(j, c):
        row_max = scores_unit(j, k_stream(j + 1))
        values_unit(j, row_max, k_stream(j + 1), v_stream(j + 1))
        return c

    lax.fori_loop(0, n_kv - 1, head, None)
    row_max = scores_unit(n_kv - 1, wo)
    values_unit(n_kv - 1, row_max, wo, shifted(wo, u))

    attn = jnp.zeros((_ROWS, d_model), f32)
    attn = run(n_q - 2 * u, shifted(wo, u), shifted(wo, 2 * u), o_proj, attn)
    attn = run(u, shifted(wo, n_q - u), w3, shifted(o_proj, n_q - 2 * u), attn)
    attn = run(u, w3, shifted(w3, u), shifted(o_proj, n_q - u), attn)
    base = gate * attn[0:1] + (1.0 - gate) * x

    half = u // 2
    run(2 * u, shifted(w3, u), shifted(w3, 2 * u), ff_up)
    run(half, shifted(w3, 3 * u), shifted(w3, 4 * u), shifted(ff_up, 2 * u))
    run(half, shifted(w3, 3 * u + half), w4, shifted(ff_up, 2 * u + half))
    run(half, shifted(w3, 4 * u), shifted(w4, half), shifted(ff_up, 3 * u))
    run(half, w4, shifted(w4, u), shifted(ff_up, 3 * u + half))
    run(half, shifted(w4, half), shifted(w4, u + half), shifted(ff_up, 4 * u))
    ff = jnp.zeros((_ROWS, d_model), f32)
    ff = run(u + half, shifted(w4, u), shifted(w4, 2 * u), ff_down, ff)
    for g in range(len(tail_groups)):
        tail_copy(g).start(priority=1)
    ff = run(u, shifted(w4, 2 * u + half), None, shifted(ff_down, u + half), ff)

    def ff_down_block(lo, n, acc):
        h = jnp.concatenate([h_s[lo + i] for i in range(n)], axis=-1).astype(bf16)
        return acc + _dot_nt(h, w4_v[:, lo * _LANES:(lo + n) * _LANES])

    ff = ff_down_block(2 * u + half, u, ff)
    lo = n_ff - u
    for g, n in enumerate(tail_groups):
        tail_copy(g).wait()
        ff = ff_down_block(lo, n, ff)
        lo += n
    o_ref[0] = (base + (1.0 - gate) * ff[0:1]).astype(o_ref.dtype)


def make(kv_side=128, w_side=128, tail_groups=(4, 2, 1, 1), **cp):
    def fn(A_x, A_k_cache, A_v_cache, A_wq, A_wo, B_x, B_w1, B_w2, B_w3, B_w4, gate_w):
        _, _, d_model = A_x.shape
        _, n_kv, s_k, d_head = A_k_cache.shape
        d_ff = B_w3.shape[1]
        window = min(4096, max(256, s_k // 4))
        bf16, f32 = jnp.bfloat16, jnp.float32
        hbm = pl.BlockSpec(memory_space=pltpu.HBM)
        return pl.pallas_call(
            functools.partial(_kernel, window=window, kv_side=kv_side, w_side=w_side, tail_groups=tail_groups),
            out_shape=jax.ShapeDtypeStruct(A_x.shape, A_x.dtype),
            in_specs=[hbm] * 8,
            scratch_shapes=[
                pltpu.VMEM((1, d_model), bf16),
                pltpu.VMEM((d_model,), bf16),
                pltpu.VMEM((n_kv, window, d_head), bf16),
                pltpu.VMEM((n_kv, window, d_head), bf16),
                pltpu.VMEM((d_model, _HQ * d_head), bf16),
                pltpu.VMEM((d_model, _HQ * d_head), bf16),
                pltpu.VMEM((d_model, d_ff), bf16),
                pltpu.VMEM((d_model, d_ff), bf16),
                pltpu.VMEM((_HQ, _ROWS, _LANES), f32),
                pltpu.VMEM((_UNIT, _ROWS, window // _UNIT), f32),
                pltpu.VMEM((_HQ, _ROWS, _LANES), f32),
                pltpu.VMEM((d_ff // _LANES, _ROWS, _LANES), f32),
                pltpu.SemaphoreType.DMA((2,)),
                pltpu.SemaphoreType.DMA((2,)),
                pltpu.SemaphoreType.DMA((len(tail_groups),)),
            ],
            compiler_params=pltpu.CompilerParams(vmem_limit_bytes=100 * 2**20, **cp),
        )(A_x, gate_w, A_k_cache, A_v_cache, A_wq, A_wo.T, B_w3, B_w4.T)
    return fn


@jax.jit
def pallas_gated_mix__sliding_block_cached__mixer_s_mlp__decode_kernel(
    A_x, A_k_cache, A_v_cache, A_wq, A_wo, B_x, B_w1, B_w2, B_w3, B_w4, gate_w
):
    return make()(A_x, A_k_cache, A_v_cache, A_wq, A_wo, B_x, B_w1, B_w2, B_w3, B_w4, gate_w)
```

```python
import functools

import jax
import jax.numpy as jnp
from jax import lax
import jax.experimental.pallas as pl
import jax.experimental.pallas.tpu as pltpu

_Q_HEADS = 32
_LANES = 128
_ROWS = 8
_UNIT_LOG2 = 3
_UNIT = 1 << _UNIT_LOG2
_KV_SIDE_ROWS = 192
_W_SIDE_ROWS = 128
_TAIL_GROUPS = (5, 2, 1)

_BULK_SEM, _SIDE_SEM = 0, 2
_BULK_PRIORITY, _SIDE_PRIORITY = 1, 0


def _dot(a, b):
    return jnp.dot(a, b, preferred_element_type=jnp.float32)


def _dot_nt(a, b):
    return lax.dot_general(
        a, b, (((1,), (1,)), ((), ())), preferred_element_type=jnp.float32
    )


def _hinted(start, multiple):
    return start if isinstance(start, int) else pl.multiple_of(start, multiple)


def _block(i, size):
    return pl.ds(_hinted(i * size, size), size)


def _lane_tiles(a):
    return [a[:, i:i + _LANES] for i in range(0, a.shape[1], _LANES)]


def _shifted(fn, offset):
    return lambda t, *rest: fn(t + offset, *rest)


def _kernel(
    x_hbm, gate_w_hbm, k_hbm, v_hbm, wq_hbm, wo_hbm, w3_hbm, w4_hbm,
    out_ref,
    x_v, gate_w_v, k_v, v_v, wq_v, wo_v, w3_v, w4_v,
    q_s, scores_s, o_s, h_s, sems,
):
    bf16, f32 = jnp.bfloat16, jnp.float32
    n_kv, window, _ = k_v.shape
    window_start = k_hbm.shape[2] - window
    d_model, d_ff = w3_hbm.shape
    ff_tiles = d_ff // _LANES
    kv_step = window // _UNIT
    scale = _LANES ** -0.5
    u, half = _UNIT, _UNIT // 2

    def kv_stream(src, dst, parity, j):
        def copy(first_row, rows, sem, s):
            row = _hinted(first_row + s * rows, 8)
            return pltpu.make_async_copy(
                src.at[0, j, pl.ds(window_start + row, rows), :],
                dst.at[j, pl.ds(row, rows), :],
                sems.at[sem + parity],
            )

        bulk_rows = kv_step - _KV_SIDE_ROWS
        return lambda s: (
            functools.partial(copy, 0, bulk_rows, _BULK_SEM, s),
            functools.partial(copy, u * bulk_rows, _KV_SIDE_ROWS, _SIDE_SEM, s),
        )

    def weight_stream(src, dst, steps_before=0):
        def copy(first_row, rows, sem, t):
            parity = ((t + steps_before) >> _UNIT_LOG2) & 1
            block = (pl.ds(first_row, rows), _block(t, _LANES))
            return pltpu.make_async_copy(
                src.at[block], dst.at[block], sems.at[sem + parity]
            )

        bulk_rows = d_model - _W_SIDE_ROWS
        return lambda t: (
            functools.partial(copy, 0, bulk_rows, _BULK_SEM, t),
            functools.partial(copy, bulk_rows, _W_SIDE_ROWS, _SIDE_SEM, t),
        )

    k_stream = functools.partial(kv_stream, k_hbm, k_v, 0)
    v_stream = functools.partial(kv_stream, v_hbm, v_v, 1)
    wq = weight_stream(wq_hbm, wq_v)
    wo = weight_stream(wo_hbm, wo_v)
    w3 = weight_stream(w3_hbm, w3_v)
    w4 = weight_stream(w4_hbm, w4_v, steps_before=ff_tiles)

    def run(steps, landing, issuing, compute=None, carry=None):
        def body(t, c):
            for copy in landing(t):
                copy().wait()
            if issuing is not None:
                bulk, side = issuing(t)
                side().start(priority=_SIDE_PRIORITY)
                bulk().start(priority=_BULK_PRIORITY)
            return c if compute is None else compute(t, c)

        return lax.fori_loop(0, steps, body, carry)

    small_copies = [
        pltpu.make_async_copy(x_hbm.at[0], x_v, sems.at[_SIDE_SEM + 1]),
        pltpu.make_async_copy(gate_w_hbm, gate_w_v, sems.at[_SIDE_SEM + 1]),
    ]
    first_unit = [wq(t) for t in range(u)]
    for bulk, _ in first_unit:
        bulk().start(priority=_BULK_PRIORITY)
    for cp in small_copies:
        cp.start(priority=_SIDE_PRIORITY)
    for _, side in first_unit:
        side().start(priority=_SIDE_PRIORITY)
    for cp in small_copies:
        cp.wait()
    run(u, wq, _shifted(wq, u))

    x = x_v[...].astype(f32)
    gate_w = gate_w_v[...].astype(f32).reshape(1, d_model)
    gate = jax.nn.sigmoid(jnp.sum(x * gate_w, axis=-1, keepdims=True))
    centered = x - jnp.mean(x, axis=-1, keepdims=True)
    var = jnp.mean(centered * centered, axis=-1, keepdims=True)
    normed = centered / jnp.sqrt(var + 1e-5)
    x_rows = jnp.broadcast_to(x, (_ROWS, d_model)).astype(bf16)
    normed_rows = jnp.broadcast_to(normed, (_ROWS, d_model)).astype(bf16)

    def q_proj(head, c):
        q_s[head] = _dot(x_rows, wq_v[:, _block(head, _LANES)])
        return c

    even_row = lax.broadcasted_iota(jnp.int32, (_ROWS, _LANES), 0) % 2 == 0

    def attend(j, following, after_following):
        q = jnp.where(even_row, q_s[2 * j], q_s[2 * j + 1]).astype(bf16)

        def qk(s, running_max):
            scores = _dot_nt(q, k_v[j, _block(s, kv_step), :])
            scores_s[s] = scores
            return functools.reduce(jnp.maximum, _lane_tiles(scores), running_max)

        lowest = jnp.full((_ROWS, _LANES), -jnp.inf, f32)
        lane_max = run(u, v_stream(j), following, qk, lowest)
        row_max = jnp.max(lane_max, axis=-1, keepdims=True)

        def pv(s, c):
            denom, acc = c
            p = jnp.exp((scores_s[s] - row_max) * scale)
            denom = functools.reduce(jnp.add, _lane_tiles(p), denom)
            return denom, acc + _dot(p.astype(bf16), v_v[j, _block(s, kv_step), :])

        zeros = jnp.zeros((_ROWS, _LANES), f32)
        denom, acc = run(u, following, after_following, pv, (zeros, zeros))
        o = acc / jnp.sum(denom, axis=-1, keepdims=True)
        o_s[2 * j] = jnp.broadcast_to(o[0:1], (_ROWS, _LANES))
        o_s[2 * j + 1] = jnp.broadcast_to(o[1:2], (_ROWS, _LANES))

    def o_proj(head, acc):
        return acc + _dot_nt(o_s[head].astype(bf16), wo_v[:, _block(head, _LANES)])

    def ff_up(t, c):
        pre = _dot(normed_rows, w3_v[:, _block(t, _LANES)])
        h_s[t] = jax.nn.gelu(pre, approximate=True)
        return c

    def ff_down(t, acc):
        return acc + _dot_nt(h_s[t].astype(bf16), w4_v[:, _block(t, _LANES)])

    def ff_down_group(first, tiles):
        h = jnp.concatenate([h_s[first + i] for i in range(tiles)], axis=-1)
        cols = pl.ds(first * _LANES, tiles * _LANES)
        return _dot_nt(h.astype(bf16), w4_v[:, cols])

    run(_Q_HEADS - 2 * u, _shifted(wq, u), _shifted(wq, 2 * u), q_proj)
    run(u, _shifted(wq, _Q_HEADS - u), k_stream(0), _shifted(q_proj, _Q_HEADS - 2 * u))
    run(u, k_stream(0), v_stream(0), _shifted(q_proj, _Q_HEADS - u))

    def head_pair(j, c):
        attend(j, k_stream(j + 1), v_stream(j + 1))
        return c

    lax.fori_loop(0, n_kv - 1, head_pair, None)
    attend(n_kv - 1, wo, _shifted(wo, u))

    attn = jnp.zeros((_ROWS, d_model), f32)
    attn = run(_Q_HEADS - 2 * u, _shifted(wo, u), _shifted(wo, 2 * u), o_proj, attn)
    attn = run(u, _shifted(wo, _Q_HEADS - u), w3, _shifted(o_proj, _Q_HEADS - 2 * u), attn)
    attn = run(u, w3, _shifted(w3, u), _shifted(o_proj, _Q_HEADS - u), attn)
    partial_out = gate * attn[0:1] + (1.0 - gate) * x

    run(2 * u, _shifted(w3, u), _shifted(w3, 2 * u), ff_up)
    run(half, _shifted(w3, 3 * u), _shifted(w3, 4 * u), _shifted(ff_up, 2 * u))
    run(half, _shifted(w3, 3 * u + half), w4, _shifted(ff_up, 2 * u + half))
    run(half, _shifted(w3, 4 * u), _shifted(w4, half), _shifted(ff_up, 3 * u))
    run(half, w4, _shifted(w4, u), _shifted(ff_up, 3 * u + half))
    run(half, _shifted(w4, half), _shifted(w4, u + half), _shifted(ff_up, 4 * u))
    ff = jnp.zeros((_ROWS, d_model), f32)
    ff = run(u + half, _shifted(w4, u), _shifted(w4, 2 * u), ff_down, ff)

    tail_sems = (_BULK_SEM, _SIDE_SEM, _BULK_SEM + 1)
    tail_starts = [ff_tiles - u + sum(_TAIL_GROUPS[:g]) for g in range(len(_TAIL_GROUPS))]
    tail_copies = []
    for first, tiles, sem in zip(tail_starts, _TAIL_GROUPS, tail_sems, strict=True):
        cols = pl.ds(first * _LANES, tiles * _LANES)
        tail_copies.append(
            pltpu.make_async_copy(w4_hbm.at[:, cols], w4_v.at[:, cols], sems.at[sem])
        )
    for cp in tail_copies[:2]:
        cp.start(priority=_BULK_PRIORITY)
    ff = run(u, _shifted(w4, 2 * u + half), None, _shifted(ff_down, u + half), ff)
    tail_copies[2].start(priority=_BULK_PRIORITY)

    ff = ff + ff_down_group(2 * u + half, u)
    for cp, first, tiles in zip(tail_copies, tail_starts, _TAIL_GROUPS, strict=True):
        cp.wait()
        ff = ff + ff_down_group(first, tiles)
    out_ref[0] = (partial_out + (1.0 - gate) * ff[0:1]).astype(out_ref.dtype)


@jax.jit
def pallas_gated_mix__sliding_block_cached__mixer_s_mlp__decode_kernel(
    A_x: jax.Array,
    A_k_cache: jax.Array,
    A_v_cache: jax.Array,
    A_wq: jax.Array,
    A_wo: jax.Array,
    B_x: jax.Array,
    B_w1: jax.Array,
    B_w2: jax.Array,
    B_w3: jax.Array,
    B_w4: jax.Array,
    gate_w: jax.Array,
):
    del B_x, B_w1, B_w2
    batch, tokens, d_model = A_x.shape
    _, n_kv, s_k, d_head = A_k_cache.shape
    d_ff = B_w3.shape[1]
    window = min(4096, max(256, s_k // 4))
    assert (batch, tokens) == (1, 1)
    assert d_head == _LANES and _Q_HEADS == 2 * n_kv
    assert d_ff == (4 * _UNIT + _UNIT // 2) * _LANES and sum(_TAIL_GROUPS) == _UNIT
    assert window % (_UNIT * _LANES) == 0 and window // _UNIT > _KV_SIDE_ROWS

    bf16, f32 = jnp.bfloat16, jnp.float32
    return pl.pallas_call(
        _kernel,
        out_shape=jax.ShapeDtypeStruct(A_x.shape, A_x.dtype),
        in_specs=[pl.BlockSpec(memory_space=pltpu.HBM)] * 8,
        scratch_shapes=[
            pltpu.VMEM((1, d_model), bf16),
            pltpu.VMEM((d_model,), bf16),
            pltpu.VMEM((n_kv, window, d_head), bf16),
            pltpu.VMEM((n_kv, window, d_head), bf16),
            pltpu.VMEM((d_model, _Q_HEADS * d_head), bf16),
            pltpu.VMEM((d_model, _Q_HEADS * d_head), bf16),
            pltpu.VMEM((d_model, d_ff), bf16),
            pltpu.VMEM((d_model, d_ff), bf16),
            pltpu.VMEM((_Q_HEADS, _ROWS, _LANES), f32),
            pltpu.VMEM((_UNIT, _ROWS, window // _UNIT), f32),
            pltpu.VMEM((_Q_HEADS, _ROWS, _LANES), f32),
            pltpu.VMEM((d_ff // _LANES, _ROWS, _LANES), f32),
            pltpu.SemaphoreType.DMA((4,)),
        ],
        compiler_params=pltpu.CompilerParams(vmem_limit_bytes=100 * 2**20),
    )(A_x, gate_w, A_k_cache, A_v_cache, A_wq, A_wo.T, B_w3, B_w4.T)
```
